```python
import os as _os
_os.environ.setdefault("JAX_PLATFORMS", "cpu")
import jax
import jax.numpy as jnp

def _softmax(x, axis=-1):
    return jax.nn.softmax(x, axis=axis)
def _gelu(x):
    return jax.nn.gelu(x, approximate=True)
def _silu(x):
    return jax.nn.silu(x)
def _sigmoid(x):
    return jax.nn.sigmoid(x)
def _layernorm(x, axis=-1, eps=1e-5):
    m = jnp.mean(x, axis=axis, keepdims=True)
    v = jnp.var(x, axis=axis, keepdims=True)
    return (x - m) / jnp.sqrt(v + eps)
def _scatter_add(tgt, idx, src, axis=0):
    return tgt.at[idx].add(src)
def _segment_sum(src, seg, n):
    return jax.ops.segment_sum(src, seg, n)
class _Rng:
    def __init__(self, key):
        self._k = key
    def _next(self):
        self._k, sub = jax.random.split(self._k)
        return sub
    def normal(self, shape):
        return jax.random.normal(self._next(), shape, dtype=jnp.bfloat16)
    def randint(self, lo, hi, shape):
        return jax.random.randint(self._next(), shape, lo, hi, dtype=jnp.int32)
    def uniform(self, shape, lo=0.0, hi=1.0):
        return jax.random.uniform(self._next(), shape, jnp.bfloat16, lo, hi)
    def permutation(self, n):
        return jax.random.permutation(self._next(), n)


kernel_name = 'concat_heads__mha_block__ssm_conv_s4__prompt'

def setup_inputs():
    _rng = _Rng(jax.random.key(int.from_bytes(__import__("os").urandom(4), "little")))
    _w = (lambda a: (lambda t: t.astype(jnp.bfloat16) if jnp.issubdtype(t.dtype, jnp.floating) else t)(jnp.asarray(a)))
    def _A_setup():
        B, S, D, H = 1, 2048, 448, 16
        return {
            "x": _w((lambda *s: _rng.normal(s) * 0.2)(B, S, D)),
            "wqkv": _w((lambda *s: _rng.normal(s) * 0.2)(D, 3 * D)),
            "wo": _w((lambda *s: _rng.normal(s) * 0.05)(D, D)),
        }
    _A_in = _A_setup()

    def _B_setup():
        B, L, D, N = 1, 2048, 448, 256
        A_re = -jnp.exp((lambda *s: _rng.normal(s) * 0.2)(D, N))
        A_im = jnp.pi * (lambda *s: _rng.normal(s) * 0.2)(D, N)
        B_re = (lambda *s: _rng.normal(s) * 0.2)(D, N)
        B_im = (lambda *s: _rng.normal(s) * 0.2)(D, N)
        C_re = (lambda *s: _rng.normal(s) * 0.2)(D, N)
        C_im = (lambda *s: _rng.normal(s) * 0.2)(D, N)
        log_dt = (lambda *s: _rng.normal(s) * 0.2)(D) * 0.5 - 4.0
        Dskip = (lambda *s: _rng.normal(s) * 0.05)(D)
        return {
            "u": _w((lambda *s: _rng.normal(s) * 0.05)(B, L, D)),
            "A_re": _w(A_re),
            "A_im": _w(A_im),
            "B_re": _w(B_re),
            "B_im": _w(B_im),
            "C_re": _w(C_re),
            "C_im": _w(C_im),
            "log_dt": _w(log_dt),
            "Dskip": _w(Dskip),
        }
    _B_in = _B_setup()

    return {
        "A_x": _A_in["x"],
        "A_wqkv": _A_in["wqkv"],
        "A_wo": _A_in["wo"],
        "B_u": _B_in["u"],
        "B_A_re": _B_in["A_re"],
        "B_A_im": _B_in["A_im"],
        "B_B_re": _B_in["B_re"],
        "B_B_im": _B_in["B_im"],
        "B_C_re": _B_in["C_re"],
        "B_C_im": _B_in["C_im"],
        "B_log_dt": _B_in["log_dt"],
        "B_Dskip": _B_in["Dskip"],
    }

def reference(A_x, A_wqkv, A_wo, B_u, B_A_re, B_A_im, B_B_re, B_B_im, B_C_re, B_C_im, B_log_dt, B_Dskip):
    def _A_ref(x, wqkv, wo):
        B, S, D = x.shape
        H = 16
        Dh = D // H
        qkv = (lambda x, *d: x.transpose(*d))((x @ wqkv).reshape(B, S, 3, H, Dh), 2, 0, 3, 1, 4)
        q, k, v = qkv[0], qkv[1], qkv[2]
        scores = jnp.einsum("bhqd,bhkd->bhqk", q, k) * (Dh ** -0.5)
        p = _softmax(scores, axis=-1)
        o = jnp.einsum("bhqk,bhkd->bhqd", p, v)
        return (lambda x, *d: x.transpose(*d))(o, 0, 2, 1, 3).reshape(B, S, D) @ wo

    def _B_ref(u, A_re, A_im, B_re, B_im, C_re, C_im, log_dt, Dskip):
        Bsz, L, D = u.shape
        dt = jnp.exp(log_dt)[:, None]
        A = A_re + 1j * A_im
        Bc = B_re + 1j * B_im
        Cc = C_re + 1j * C_im
        logdA = dt * A
        dB = dt * Bc
        l = (lambda x, dt: x.astype(dt))(jnp.arange(L), A_re.dtype)
        P = jnp.exp(logdA[:, :, None] * l[None, None, :])
        K = jnp.einsum("dn,dnl,dn->dl", Cc, P, dB).real
        L2 = 2 * L
        Kp = jnp.pad(K, ((0, 0), (0, L)))
        up = (lambda x, *d: x.transpose(*d))(u, 0, 2, 1)
        up = jnp.pad(up, ((0, 0), (0, 0), (0, L)))
        Kf = (lambda x, axes=(-2,-1): jnp.fft.rfft2(x.astype(jnp.float32), axes=axes))(Kp[:, None, :], axes=(-2, -1))
        Uf = (lambda x, axes=(-2,-1): jnp.fft.rfft2(x.astype(jnp.float32), axes=axes))(up[:, :, None, :], axes=(-2, -1))
        Yf = Uf * Kf[None, :, :, :]
        y = (lambda x, s, axes=(-2,-1): jnp.fft.irfft2(x, s=s, axes=axes).astype(jnp.bfloat16))(Yf, (1, L2), axes=(-2, -1))[:, :, 0, :L]
        y = (lambda x, *d: x.transpose(*d))(y, 0, 2, 1) + u * Dskip[None, None, :]
        return y

    a = _A_ref(A_x, A_wqkv, A_wo)
    b = _B_ref(B_u, B_A_re, B_A_im, B_B_re, B_B_im, B_C_re, B_C_im, B_log_dt, B_Dskip)
    return jnp.concatenate([a, b], axis=-1)
```

```python
import functools
import math

import numpy as np
import jax
import jax.numpy as jnp
from jax import lax
import jax.experimental.pallas as pl
import jax.experimental.pallas.tpu as pltpu

S = 2048
D = 448
H = 16
DH = 28
DHP = 32
NST = 256
CH = 128
NCH = S // CH
FP = 136
TQ = 256
DB = 64
XR = 48
ZR = 128


def _bf16_round_int(l):
    l = np.asarray(l, dtype=np.int64)
    out = np.empty_like(l)
    for idx, v in enumerate(l.ravel()):
        v = int(v)
        if v < 256:
            out.ravel()[idx] = v
            continue
        s = 1 << (v.bit_length() - 8)
        q, rem = divmod(v, s)
        if rem * 2 > s or (rem * 2 == s and (q & 1)):
            q += 1
        out.ravel()[idx] = q * s
    return out


def _x_rows():
    rows = []
    for a in range(16):
        rows.append((16 * a, 0))
    for a in range(8):
        rows.append((256 + 32 * a, 1))
    for a in range(8):
        rows.append((512 + 64 * a, 2))
    for a in range(8):
        rows.append((1024 + 128 * a, 3))
    rows.append((2048, 3))
    return rows


@functools.lru_cache(maxsize=None)
def _build_tables():
    f = np.arange(FP)[:, None]
    valid = (f < 129).astype(np.float64)
    i = np.arange(CH)[None, :]
    ang = 2.0 * np.pi * ((f * i) % 256) / 256.0
    fu = np.concatenate([np.cos(ang) * valid, -np.sin(ang) * valid], axis=0)

    t = np.arange(256)[:, None]
    ff = np.arange(FP)[None, :]
    w = np.where((ff == 0) | (ff == 128), 1.0, 2.0) * (ff < 129) / 256.0
    ang = 2.0 * np.pi * ((t * ff) % 256) / 256.0
    g = np.concatenate([np.cos(ang) * w, -np.sin(ang) * w], axis=1)

    rl = _bf16_round_int(np.arange(S))
    rows = _x_rows()
    mats, pairs = [], []
    for k in range(NCH):
        for r, (e, grp) in enumerate(rows):
            s = 1 << grp
            mat = np.zeros((2 * FP, 128), np.float64)
            used = False
            for b in range(16):
                m = e + s * b
                if r == 40 and b > 0:
                    continue
                ls = [l for l in range(CH * k, CH * k + CH) if rl[l] == m]
                for l in ls:
                    used = True
                    a2 = 2.0 * np.pi * ((np.arange(FP) * (l - CH * k)) % 256) / 256.0
                    v = (np.arange(FP) < 129)
                    mat[:FP, b * 8:(b + 1) * 8] += (np.cos(a2) * v)[:, None]
                    mat[FP:, b * 8:(b + 1) * 8] += (-np.sin(a2) * v)[:, None]
            if used:
                mats.append(mat)
                pairs.append((k, r))
    ffold = np.stack(mats)
    return (fu.astype(np.float32), g.astype(np.float32), ffold.astype(np.float32),
            tuple(pairs))


def _cmul(ar, ai, br, bi):
    return ar * br - ai * bi, ar * bi + ai * br


def _kgen(are_ref, aim_ref, bre_ref, bim_ref, cre_ref, cim_ref, ldt_ref,
          x_s, z_s, kt_s):
    f32 = jnp.float32
    bf16 = jnp.bfloat16
    xrows = _x_rows()
    def per_block(db, carry0):
        dr = pl.ds(pl.multiple_of(db * DB, DB), DB)
        dt = jnp.exp(ldt_ref[dr, :].astype(f32)).astype(bf16).astype(f32)
        al = dt * are_ref[dr, :].astype(f32)
        om = dt * aim_ref[dr, :].astype(f32)
        dbr = dt * bre_ref[dr, :].astype(f32)
        dbi = dt * bim_ref[dr, :].astype(f32)
        cr, ci = _cmul(cre_ref[dr, :].astype(f32), cim_ref[dr, :].astype(f32), dbr, dbi)

        def zpow(e):
            mag = jnp.exp(al * e)
            return mag * jnp.cos(om * e), mag * jnp.sin(om * e)

        one = jnp.ones((DB, NST), f32)
        zero = jnp.zeros((DB, NST), f32)

        def chain(base, n):
            out = [(one, zero), base]
            for _ in range(2, n):
                out.append(_cmul(out[-1][0], out[-1][1], base[0], base[1]))
            return out

        t0 = chain(zpow(1.0), 16)
        t1 = chain(zpow(16.0), 16)
        t2 = chain(zpow(256.0), 9)

        def zp(e):
            e2, rem = divmod(e, 256)
            e1, e0 = divmod(rem, 16)
            fac = [tb[j] for tb, j in ((t2, e2), (t1, e1), (t0, e0)) if j]
            if not fac:
                return one, zero
            acc = fac[0]
            for fc in fac[1:]:
                acc = _cmul(acc[0], acc[1], fc[0], fc[1])
            return acc

        for grp in range(4):
            for b in range(16):
                vr, vi = zp((1 << grp) * b)
                z_s[grp * 16 + b] = jnp.concatenate([vr, vi], axis=1).astype(bf16)
        for r, (e, _) in enumerate(xrows):
            pr, pi_ = zp(e)
            vr, vi = _cmul(cr, ci, pr, pi_)
            x_s[r] = jnp.concatenate([vr, -vi], axis=1).astype(bf16)

        sub = lax.broadcasted_iota(jnp.int32, (8, 128), 0)
        lane = lax.broadcasted_iota(jnp.int32, (8, 128), 1)
        diag = (lane % 8) == sub
        grp_rows = [[r for r, (_, g) in enumerate(xrows) if g == grp] for grp in range(4)]

        def per_group(gi, carry):
            row0 = pl.multiple_of(gi * 8, 8)
            out0 = pl.multiple_of(db * DB + gi * 8, 8)
            for grp in range(4):
                rs = grp_rows[grp]
                lhs = jnp.concatenate([x_s[r, pl.ds(row0, 8), :] for r in rs], axis=0)
                rhs = jnp.concatenate(
                    [z_s[grp * 16 + b, pl.ds(row0, 8), :] for b in range(16)], axis=0)
                o = lax.dot_general(lhs, rhs, (((1,), (1,)), ((), ())),
                                    preferred_element_type=f32)
                for idx, r in enumerate(rs):
                    blk = o[idx * 8:(idx + 1) * 8]
                    kt_s[r, pl.ds(out0, 8), :] = jnp.where(diag, blk, 0.0).astype(bf16)
            return carry

        lax.fori_loop(0, DB // 8, per_group, 0)
        return carry0

    lax.fori_loop(0, D // DB, per_block, 0)


def _kernel(pairs,
            x_ref, wqkv_ref, wo_ref, u_ref, are_ref, aim_ref, bre_ref, bim_ref,
            cre_ref, cim_ref, ldt_ref, dsk_ref, fu_ref, g_ref, ff_ref,
            o_ref,
            qkv_s, ot_s, x_s, z_s, kt_s, kf_s, uf_s, yf_s, yb_s):
    step = pl.program_id(0)
    f32 = jnp.float32
    bf16 = jnp.bfloat16

    @pl.when(step == 0)
    def _prologue():
        with jax.named_scope('qkv'):
          for rb in range(S // 512):
            rows = pl.ds(rb * 512, 512)
            qkv = jnp.dot(x_ref[rows, :], wqkv_ref[...], preferred_element_type=f32)
            lane = lax.broadcasted_iota(jnp.int32, qkv.shape, 1)
            is_vpad = (lane >= 2 * 512) & ((lane % DHP) >= DH)
            qkv = jnp.where(is_vpad, 1.0, qkv)
            for t in range(12):
                qkv_s[t, rows, :] = qkv[:, 128 * t:128 * (t + 1)].astype(bf16)

        with jax.named_scope("kgen"):
            _kgen(are_ref, aim_ref, bre_ref, bim_ref, cre_ref, cim_ref, ldt_ref,
                  x_s, z_s, kt_s)

        with jax.named_scope("dft"):
            by_chunk = {}
            for p, (k, r) in enumerate(pairs):
                by_chunk.setdefault(k, []).append((p, r))
            for k in range(NCH):
                acc = None
                for (p, r) in by_chunk[k]:
                    t = lax.dot_general(ff_ref[p], kt_s[r], (((1,), (1,)), ((), ())),
                                        preferred_element_type=f32)
                    acc = t if acc is None else acc + t
                kf_s[k] = acc
                uf_s[k] = jnp.dot(fu_ref[...], u_ref[pl.ds(k * CH, CH), :],
                                  preferred_element_type=f32)

        with jax.named_scope("freq"):
            tail = jnp.zeros((CH, D), f32)
            for c in range(NCH):
                def rb_body(rb, carry, c=c):
                    r0 = pl.multiple_of(rb * 8, 8)
                    r1 = pl.multiple_of(rb * 8 + FP, 8)

                    def acc_body(k, acc):
                        yr, yi = acc
                        ur = uf_s[c - k, pl.ds(r0, 8), :]
                        ui = uf_s[c - k, pl.ds(r1, 8), :]
                        kr = kf_s[k, pl.ds(r0, 8), :]
                        ki = kf_s[k, pl.ds(r1, 8), :]
                        return yr + (ur * kr - ui * ki), yi + (ur * ki + ui * kr)

                    z = jnp.zeros((8, D), f32)
                    yr, yi = lax.fori_loop(0, c + 1, acc_body, (z, z))
                    yf_s[pl.ds(r0, 8), :] = yr
                    yf_s[pl.ds(r1, 8), :] = yi
                    return carry

                lax.fori_loop(0, FP // 8, rb_body, 0)
                yc = jnp.dot(g_ref[...], yf_s[...].astype(bf16),
                             preferred_element_type=f32)
                y = yc[:CH] + tail
                tail = yc[CH:]
                rows = pl.ds(c * CH, CH)
                skip = (u_ref[rows, :].astype(f32) * dsk_ref[...].astype(f32)).astype(bf16)
                yb_s[rows, :] = (y.astype(bf16).astype(f32) + skip.astype(f32)).astype(bf16)

    qrows = pl.ds(pl.multiple_of(step * TQ, TQ), TQ)
    cexp = (DH ** -0.5) * math.log2(math.e)
    lane = lax.broadcasted_iota(jnp.int32, (TQ, 128), 1)
    with jax.named_scope('attn'):
        def tile_body(t, carry):
            qt = qkv_s[t, qrows, :]
            kt = qkv_s[4 + t]
            vt = qkv_s[8 + t]
            ot = jnp.zeros((TQ, 128), f32)
            for j in range(4):
                in_head = (lane // DHP) == j
                qm = jnp.where(in_head, qt, jnp.zeros_like(qt))
                s = lax.dot_general(qm, kt, (((1,), (1,)), ((), ())),
                                    preferred_element_type=f32)
                m = jnp.max(s, axis=1, keepdims=True)
                p = jnp.exp2((s - m) * cexp).astype(bf16)
                o = jnp.dot(p, vt, preferred_element_type=f32)
                l = jnp.sum(jnp.where(lane == DH, o, 0.0), axis=1, keepdims=True)
                ot = jnp.where(in_head, o / l, ot)
            ot_s[t] = ot.astype(bf16)
            return carry

        lax.fori_loop(0, 4, tile_body, 0)
    oall = jnp.concatenate([ot_s[t] for t in range(4)], axis=1)
    a = jnp.dot(oall, wo_ref[...], preferred_element_type=f32).astype(bf16)
    o_ref[:, pl.ds(0, D)] = a
    o_ref[:, pl.ds(D, D)] = yb_s[qrows, :]


@jax.jit
def pallas_concat_heads__mha_block__ssm_conv_s4__prompt_kernel(
    A_x: jax.Array,
    A_wqkv: jax.Array,
    A_wo: jax.Array,
    B_u: jax.Array,
    B_A_re: jax.Array,
    B_A_im: jax.Array,
    B_B_re: jax.Array,
    B_B_im: jax.Array,
    B_C_re: jax.Array,
    B_C_im: jax.Array,
    B_log_dt: jax.Array,
    B_Dskip: jax.Array,
):
    bf16 = jnp.bfloat16
    x = A_x.reshape(S, D)
    wqkv = jnp.pad(A_wqkv.reshape(D, 3, H, DH), ((0, 0), (0, 0), (0, 0), (0, DHP - DH)))
    wqkv = wqkv.reshape(D, 3 * H * DHP)
    wo = jnp.pad(A_wo.reshape(H, DH, D), ((0, 0), (0, DHP - DH), (0, 0))).reshape(H * DHP, D)
    u = B_u.reshape(S, D)
    ldt = B_log_dt.reshape(D, 1)
    dsk = B_Dskip.reshape(1, D)

    fu, g, ffold, pairs = _build_tables()
    fu = jnp.asarray(fu, dtype=bf16)
    g = jnp.asarray(g, dtype=bf16)
    ffold = jnp.asarray(ffold, dtype=bf16)

    def full(shape):
        nd = len(shape)
        return pl.BlockSpec(shape, lambda i, _nd=nd: (0,) * _nd)

    in_arrays = [x, wqkv, wo, u, B_A_re, B_A_im, B_B_re, B_B_im, B_C_re, B_C_im,
                 ldt, dsk, fu, g, ffold]
    in_specs = [full(a.shape) for a in in_arrays]

    out = pl.pallas_call(
        functools.partial(_kernel, pairs),
        grid=(S // TQ,),
        in_specs=in_specs,
        out_specs=pl.BlockSpec((TQ, 2 * D), lambda i: (i, 0)),
        out_shape=jax.ShapeDtypeStruct((S, 2 * D), bf16),
        scratch_shapes=[
            pltpu.VMEM((12, S, 128), bf16),
            pltpu.VMEM((4, TQ, 128), bf16),
            pltpu.VMEM((41, DB, 2 * NST), bf16),
            pltpu.VMEM((64, DB, 2 * NST), bf16),
            pltpu.VMEM((41, D, 128), bf16),
            pltpu.VMEM((NCH, 2 * FP, D), jnp.float32),
            pltpu.VMEM((NCH, 2 * FP, D), jnp.float32),
            pltpu.VMEM((2 * FP, D), jnp.float32),
            pltpu.VMEM((S, D), bf16),
        ],
        compiler_params=pltpu.CompilerParams(
            dimension_semantics=("arbitrary",),
            vmem_limit_bytes=100 * 1024 * 1024,
        ),
    )(*in_arrays)
    return out.reshape(1, S, 2 * D)
```

```python
import functools
import math

import numpy as np
import jax
import jax.numpy as jnp
from jax import lax
import jax.experimental.pallas as pl
import jax.experimental.pallas.tpu as pltpu

S = 2048
D = 448
H = 16
DH = 28
DHP = 32
NST = 256
CH = 128
NCH = S // CH
DFT_CLASSES = ((0, 2, 8, 0, 0, 8), (2, 2, 5, 16, 16, 4), (4, 4, 3, 26, 24, 2), (8, 8, 2, 38, 32, 1))
NPAIR = 54
TQ = 512
DB = 64
XR = 42
NG = DB // 8


def _bf16_round_int(l):
    l = np.asarray(l, dtype=np.int64)
    out = np.empty_like(l)
    for idx, v in enumerate(l.ravel()):
        v = int(v)
        if v < 256:
            out.ravel()[idx] = v
            continue
        s = 1 << (v.bit_length() - 8)
        q, rem = divmod(v, s)
        if rem * 2 > s or (rem * 2 == s and (q & 1)):
            q += 1
        out.ravel()[idx] = q * s
    return out


def _x_rows():
    rows = []
    for a in range(16):
        rows.append((16 * a, 0))
    for a in range(8):
        rows.append((256 + 32 * a, 1))
    for a in range(8):
        rows.append((512 + 64 * a, 2))
    for a in range(8):
        rows.append((1024 + 128 * a, 3))
    rows.append((2048, 3))
    return rows


@functools.lru_cache(maxsize=None)
def _build_tables():
    def basis(off):
        f = np.arange(128)
        ang = 2.0 * np.pi * ((f * off) % 256) / 256.0
        re = np.cos(ang)
        im = -np.sin(ang)
        im[0] = np.cos(np.pi * (off % 2))
        return np.concatenate([re, im])

    fu = np.stack([basis(i) for i in range(CH)], axis=1)

    t = np.arange(256)[:, None]
    ff = np.arange(128)[None, :]
    ang = 2.0 * np.pi * ((t * ff) % 256) / 256.0
    gre = 2.0 * np.cos(ang) / 256.0
    gre[:, 0] = 1.0 / 256.0
    gim = -2.0 * np.sin(ang) / 256.0
    gim[:, 0] = np.cos(np.pi * (np.arange(256) % 2)) / 256.0
    g = np.concatenate([gre, gim], axis=1)

    rl = _bf16_round_int(np.arange(S))
    rows = _x_rows()
    mats, pairs = [], []
    for k in range(NCH):
        for r, (e, grp) in enumerate(rows):
            s = 1 << grp
            mat = np.zeros((256, 128), np.float64)
            used = False
            for b in range(16):
                m = e + s * b
                if r == 40 and b > 0:
                    continue
                for l in range(CH * k, CH * k + CH):
                    if rl[l] == m:
                        used = True
                        mat[:, b * 8:(b + 1) * 8] += basis(l - CH * k)[:, None]
            if used:
                mats.append(mat)
                pairs.append((k, r))
    ffold = np.stack(mats)
    expect = [(k0 + i, r0 + rstep * i + j) for (k0, nk, cnt, p0, r0, rstep) in DFT_CLASSES
              for i in range(nk) for j in range(cnt)]
    assert expect == pairs
    return fu.astype(np.float32), g.astype(np.float32), ffold.astype(np.float32)


def _cmul(ar, ai, br, bi):
    return ar * br - ai * bi, ar * bi + ai * br


def _kgen(are_ref, aim_ref, bre_ref, bim_ref, cre_ref, cim_ref, ldt_ref,
          x_s, z_s, kt_s):
    f32 = jnp.float32
    bf16 = jnp.bfloat16
    xrows = _x_rows()
    nblk = D // DB

    def gen(db):
        dr = pl.ds(pl.multiple_of(db * DB, DB), DB)
        dt = jnp.exp(ldt_ref[dr, :].astype(f32)).astype(bf16).astype(f32)
        al = dt * are_ref[dr, :].astype(f32)
        om = dt * aim_ref[dr, :].astype(f32)
        dbr = dt * bre_ref[dr, :].astype(f32)
        dbi = dt * bim_ref[dr, :].astype(f32)
        cr, ci = _cmul(cre_ref[dr, :].astype(f32), cim_ref[dr, :].astype(f32), dbr, dbi)

        one = jnp.ones((DB, NST), f32)
        zero = jnp.zeros((DB, NST), f32)

        def chain(base, n):
            out = [(one, zero), base]
            for _ in range(2, n):
                out.append(_cmul(out[-1][0], out[-1][1], base[0], base[1]))
            return out

        def csq(a, n):
            for _ in range(n):
                a = (a[0] * a[0] - a[1] * a[1], 2.0 * a[0] * a[1])
            return a

        mag = jnp.exp(al)
        z1 = (mag * jnp.cos(om), mag * jnp.sin(om))
        z16 = csq(z1, 4)
        z256 = csq(z16, 4)
        t0 = chain(z1, 16)
        t1 = chain(z16, 16)
        t2 = chain(z256, 9)
        ct2 = [(cr, ci)] + [_cmul(cr, ci, t2[j][0], t2[j][1]) for j in range(1, 9)]

        def zrow(grp, b):
            e1, e0 = divmod((1 << grp) * b, 16)
            if e1 and e0:
                v = _cmul(t1[e1][0], t1[e1][1], t0[e0][0], t0[e0][1])
            elif e1:
                v = t1[e1]
            else:
                v = t0[e0]
            return jnp.concatenate([v[0], v[1]], axis=1).reshape(NG, 8, 2 * NST)

        def xrow(r):
            if r >= len(xrows):
                return jnp.zeros((NG, 8, 2 * NST), f32)
            e = xrows[r][0]
            e2, e1 = e // 256, (e % 256) // 16
            if e1:
                v = _cmul(ct2[e2][0], ct2[e2][1], t1[e1][0], t1[e1][1])
            else:
                v = ct2[e2]
            return jnp.concatenate([v[0], -v[1]], axis=1).reshape(NG, 8, 2 * NST)

        for grp in range(4):
            for b in range(0, 16, 2):
                z_s[:, pl.ds(grp * 128 + b * 8, 16), :] = jnp.concatenate(
                    [zrow(grp, b), zrow(grp, b + 1)], axis=1).astype(bf16)
        for r in range(0, XR, 2):
            x_s[:, pl.ds(r * 8, 16), :] = jnp.concatenate(
                [xrow(r), xrow(r + 1)], axis=1).astype(bf16)

    sub = lax.broadcasted_iota(jnp.int32, (8, 128), 0)
    lane = lax.broadcasted_iota(jnp.int32, (8, 128), 1)
    diag = (lane % 8) == sub
    grp_span = [(0, 16), (16, 8), (24, 8), (32, 10)]

    def mm(db):
        def per_group(gi, carry):
            out0 = pl.multiple_of(db * DB + gi * 8, 8)
            for grp in range(4):
                r0, nr = grp_span[grp]
                lhs = x_s[gi, pl.ds(r0 * 8, nr * 8), :]
                rhs = z_s[gi, pl.ds(grp * 128, 128), :]
                o = lax.dot_general(lhs, rhs, (((1,), (1,)), ((), ())),
                                    preferred_element_type=f32)
                for idx in range(nr):
                    if r0 + idx >= len(xrows):
                        continue
                    blk = o[idx * 8:(idx + 1) * 8]
                    kt_s[r0 + idx, pl.ds(out0, 8), :] = jnp.where(diag, blk, 0.0)
            return carry

        lax.fori_loop(0, NG, per_group, 0, unroll=8)

    def per_block(db, carry):
        gen(db)
        mm(db)
        return carry

    lax.fori_loop(0, nblk, per_block, 0)


def _kernel(xt_ref, wt_ref, wo_ref, ut_ref, are_ref, aim_ref, bre_ref, bim_ref,
            cre_ref, cim_ref, ldt_ref, dsk_ref, fu_ref, g_ref, ff_ref,
            o_ref,
            q_s, kvt_s, ot_s, x_s, z_s, kt_s, kf_s, uf_s, yf_s, tail_s, yb_s):
    step = pl.program_id(0)
    f32 = jnp.float32
    bf16 = jnp.bfloat16
    nt = (((1,), (1,)), ((), ()))

    @pl.when(step == 0)
    def _prologue():
        with jax.named_scope('qkv'):
            def qkv_body(cb, carry):
                cols = pl.ds(pl.multiple_of(cb * 512, 512), 512)
                qkv = jnp.dot(wt_ref[...], xt_ref[:, cols],
                              preferred_element_type=f32)
                for t in range(4):
                    q_s[t, cols, :] = qkv[128 * t:128 * (t + 1), :].T.astype(bf16)
                    kvt_s[t, :, cols] = qkv[512 + 128 * t:512 + 128 * (t + 1), :].astype(bf16)
                    vt = qkv[1024 + 128 * t:1024 + 128 * (t + 1), :]
                    sub = lax.broadcasted_iota(jnp.int32, vt.shape, 0)
                    vt = jnp.where((sub % DHP) >= DH, 1.0, vt)
                    kvt_s[4 + t, :, cols] = vt.astype(bf16)
                return carry

            lax.fori_loop(0, S // 512, qkv_body, 0)

        with jax.named_scope("kgen"):
            _kgen(are_ref, aim_ref, bre_ref, bim_ref, cre_ref, cim_ref, ldt_ref,
                  x_s, z_s, kt_s)

        with jax.named_scope("dft"):
            def make_body(k0, cnt, p0, r0, rstep):
                def body(i, carry):
                    k = k0 + i
                    acc = None
                    for j in range(cnt):
                        t = lax.dot_general(ff_ref[p0 + cnt * i + j],
                                            kt_s[r0 + rstep * i + j].astype(bf16), nt,
                                            preferred_element_type=f32)
                        acc = t if acc is None else acc + t
                    kf_s[k, pl.ds(0, 256), :] = acc
                    kr0 = acc[0:8]
                    ki0 = acc[128:136]
                    row0 = lax.broadcasted_iota(jnp.int32, kr0.shape, 0) == 0
                    kf_s[k, pl.ds(256, 8), :] = jnp.where(row0, 0.0, ki0)
                    kf_s[k, pl.ds(264, 8), :] = jnp.where(row0, ki0, kr0)
                    cols = pl.ds(pl.multiple_of(k * CH, CH), CH)
                    uf_s[k] = lax.dot_general(fu_ref[...], ut_ref[:, cols], nt,
                                              preferred_element_type=f32)
                    return carry
                return body

            for (k0, nk, cnt, p0, r0, rstep) in DFT_CLASSES:
                lax.fori_loop(0, nk, make_body(k0, cnt, p0, r0, rstep), 0)

        with jax.named_scope("freq"):
            def rb_body(rb, carry):
                r0 = pl.multiple_of(rb * 8, 8)
                r1 = pl.multiple_of(rb * 8 + 128, 8)
                ra = pl.multiple_of(jnp.where(rb == 0, 256, rb * 8 + 128), 8)
                rbb = pl.multiple_of(jnp.where(rb == 0, 264, rb * 8), 8)
                for c in range(NCH):
                    yr = yi = None
                    for k in range(c + 1):
                        ur = uf_s[c - k, pl.ds(r0, 8), :]
                        ui = uf_s[c - k, pl.ds(r1, 8), :]
                        kr = kf_s[k, pl.ds(r0, 8), :]
                        ka = kf_s[k, pl.ds(ra, 8), :]
                        kb = kf_s[k, pl.ds(rbb, 8), :]
                        tr = ur * kr - ui * ka
                        ti = ur * ka + ui * kb
                        yr = tr if yr is None else yr + tr
                        yi = ti if yi is None else yi + ti
                    yf_s[c, pl.ds(r0, 8), :] = yr
                    yf_s[c, pl.ds(r1, 8), :] = yi
                return carry

            lax.fori_loop(0, 16, rb_body, 0)

        with jax.named_scope("idft"):
            tail_s[...] = jnp.zeros((CH, D), f32)

            def idft_body(c, carry):
                yc = jnp.dot(g_ref[...], yf_s[c].astype(bf16),
                             preferred_element_type=f32)
                y = yc[:CH] + tail_s[...]
                tail_s[...] = yc[CH:]
                rows = pl.ds(pl.multiple_of(c * CH, CH), CH)
                uc = ut_ref[:, rows].astype(f32).T
                skip = (uc * dsk_ref[...].astype(f32)).astype(bf16)
                yb_s[rows, :] = (y.astype(bf16).astype(f32) + skip.astype(f32)).astype(bf16)
                return carry

            lax.fori_loop(0, NCH, idft_body, 0)

    qrows = pl.ds(pl.multiple_of(step * TQ, TQ), TQ)
    cexp = (DH ** -0.5) * math.log2(math.e)
    lane = lax.broadcasted_iota(jnp.int32, (TQ, 128), 1)
    with jax.named_scope('attn'):
        def tile_body(t, carry):
            qt = q_s[t, qrows, :]
            kt = kvt_s[t]
            vt = kvt_s[4 + t]
            ot = jnp.zeros((TQ, 128), f32)
            for j in range(4):
                in_head = (lane // DHP) == j
                qm = jnp.where(in_head, qt, jnp.zeros_like(qt))
                s = jnp.dot(qm, kt, preferred_element_type=f32)
                m = jnp.max(s, axis=1, keepdims=True)
                p = jnp.exp2((s - m) * cexp).astype(bf16)
                o = lax.dot_general(p, vt, (((1,), (1,)), ((), ())),
                                    preferred_element_type=f32)
                l = jnp.sum(jnp.where(lane == DH, o, 0.0), axis=1, keepdims=True)
                ot = jnp.where(in_head, o / l, ot)
            ot_s[t] = ot.astype(bf16)
            return carry

        lax.fori_loop(0, 4, tile_body, 0)
    oall = jnp.concatenate([ot_s[t] for t in range(4)], axis=1)
    a = jnp.dot(oall, wo_ref[...], preferred_element_type=f32).astype(bf16)
    o_ref[:, pl.ds(0, D)] = a
    o_ref[:, pl.ds(D, D)] = yb_s[qrows, :]


@jax.jit
def pallas_concat_heads__mha_block__ssm_conv_s4__prompt_kernel(
    A_x: jax.Array,
    A_wqkv: jax.Array,
    A_wo: jax.Array,
    B_u: jax.Array,
    B_A_re: jax.Array,
    B_A_im: jax.Array,
    B_B_re: jax.Array,
    B_B_im: jax.Array,
    B_C_re: jax.Array,
    B_C_im: jax.Array,
    B_log_dt: jax.Array,
    B_Dskip: jax.Array,
):
    bf16 = jnp.bfloat16
    xt = A_x.reshape(S, D).T
    wt = jnp.pad(A_wqkv.T.reshape(3 * H, DH, D), ((0, 0), (0, DHP - DH), (0, 0)))
    wt = wt.reshape(3 * H * DHP, D)
    wo = jnp.pad(A_wo.reshape(H, DH, D), ((0, 0), (0, DHP - DH), (0, 0))).reshape(H * DHP, D)
    ut = B_u.reshape(S, D).T
    ldt = B_log_dt.reshape(D, 1)
    dsk = B_Dskip.reshape(1, D)

    fu, g, ffold = _build_tables()
    assert ffold.shape[0] == NPAIR
    fu = jnp.asarray(fu, dtype=bf16)
    g = jnp.asarray(g, dtype=bf16)
    ffold = jnp.asarray(ffold, dtype=bf16)

    def full(shape):
        nd = len(shape)
        return pl.BlockSpec(shape, lambda i, _nd=nd: (0,) * _nd)

    in_arrays = [xt, wt, wo, ut, B_A_re, B_A_im, B_B_re, B_B_im, B_C_re, B_C_im,
                 ldt, dsk, fu, g, ffold]
    in_specs = [full(a.shape) for a in in_arrays]

    grid_spec = pltpu.PrefetchScalarGridSpec(
        num_scalar_prefetch=0,
        grid=(S // TQ,),
        in_specs=in_specs,
        out_specs=pl.BlockSpec((TQ, 2 * D), lambda i: (i, 0)),
        scratch_shapes=[
            pltpu.VMEM((4, S, 128), bf16),
            pltpu.VMEM((8, 128, S), bf16),
            pltpu.VMEM((4, TQ, 128), bf16),
            pltpu.VMEM((NG, XR * 8, 2 * NST), bf16),
            pltpu.VMEM((NG, 512, 2 * NST), bf16),
            pltpu.VMEM((41, D, 128), jnp.float32),
            pltpu.VMEM((NCH, 272, D), jnp.float32),
            pltpu.VMEM((NCH, 256, D), jnp.float32),
            pltpu.VMEM((NCH, 256, D), jnp.float32),
            pltpu.VMEM((CH, D), jnp.float32),
            pltpu.VMEM((S, D), bf16),
        ],
    )
    out = pl.pallas_call(
        _kernel,
        grid_spec=grid_spec,
        out_shape=jax.ShapeDtypeStruct((S, 2 * D), bf16),
        compiler_params=pltpu.CompilerParams(
            dimension_semantics=("arbitrary",),
            vmem_limit_bytes=100 * 1024 * 1024,
        ),
    )(*in_arrays)
    return out.reshape(1, S, 2 * D)
```
